```python
import os as _os
_os.environ.setdefault("JAX_PLATFORMS", "cpu")
import jax
import jax.numpy as jnp

def _softmax(x, axis=-1):
    return jax.nn.softmax(x, axis=axis)
def _gelu(x):
    return jax.nn.gelu(x, approximate=True)
def _silu(x):
    return jax.nn.silu(x)
def _sigmoid(x):
    return jax.nn.sigmoid(x)
def _layernorm(x, axis=-1, eps=1e-5):
    m = jnp.mean(x, axis=axis, keepdims=True)
    v = jnp.var(x, axis=axis, keepdims=True)
    return (x - m) / jnp.sqrt(v + eps)
def _scatter_add(tgt, idx, src, axis=0):
    return tgt.at[idx].add(src)
def _segment_sum(src, seg, n):
    return jax.ops.segment_sum(src, seg, n)
class _Rng:
    def __init__(self, key):
        self._k = key
    def _next(self):
        self._k, sub = jax.random.split(self._k)
        return sub
    def normal(self, shape):
        return jax.random.normal(self._next(), shape, dtype=jnp.bfloat16)
    def randint(self, lo, hi, shape):
        return jax.random.randint(self._next(), shape, lo, hi, dtype=jnp.int32)
    def uniform(self, shape, lo=0.0, hi=1.0):
        return jax.random.uniform(self._next(), shape, jnp.bfloat16, lo, hi)
    def permutation(self, n):
        return jax.random.permutation(self._next(), n)


kernel_name = 'parallel_sum__mha_block__swiglu_ffn__prompt'

def setup_inputs():
    _rng = _Rng(jax.random.key(int.from_bytes(__import__("os").urandom(4), "little")))
    _w = (lambda a: (lambda t: t.astype(jnp.bfloat16) if jnp.issubdtype(t.dtype, jnp.floating) else t)(jnp.asarray(a)))
    def _A_setup():
        B, S, D, H = 1, 2048, 640, 32
        return {
            "x": _w((lambda *s: _rng.normal(s) * 0.05)(B, S, D)),
            "wqkv": _w((lambda *s: _rng.normal(s) * 0.1)(D, 3 * D)),
            "wo": _w((lambda *s: _rng.normal(s) * 0.05)(D, D)),
        }
    _A_in = _A_setup()

    def _B_setup():
        B, S, D, F = 1, 2048, 640, 1536
        return {
            "x": _w((lambda *s: _rng.normal(s) * 0.05)(B, S, D)),
            "w_gate": _w((lambda *s: _rng.normal(s) * 0.05)(D, F)),
            "w_up": _w((lambda *s: _rng.normal(s) * 0.05)(D, F)),
            "w_down": _w((lambda *s: _rng.normal(s) * 0.05)(F, D)),
        }
    _B_in = _B_setup()

    return {
        "A_x": _A_in["x"],
        "A_wqkv": _A_in["wqkv"],
        "A_wo": _A_in["wo"],
        "B_x": _B_in["x"],
        "B_w_gate": _B_in["w_gate"],
        "B_w_up": _B_in["w_up"],
        "B_w_down": _B_in["w_down"],
    }

def reference(A_x, A_wqkv, A_wo, B_x, B_w_gate, B_w_up, B_w_down):
    def _A_ref(x, wqkv, wo):
        B, S, D = x.shape
        H = 32
        Dh = D // H
        qkv = (lambda x, *d: x.transpose(*d))((x @ wqkv).reshape(B, S, 3, H, Dh), 2, 0, 3, 1, 4)
        q, k, v = qkv[0], qkv[1], qkv[2]
        scores = jnp.einsum("bhqd,bhkd->bhqk", q, k) * (Dh ** -0.5)
        p = _softmax(scores, axis=-1)
        o = jnp.einsum("bhqk,bhkd->bhqd", p, v)
        return (lambda x, *d: x.transpose(*d))(o, 0, 2, 1, 3).reshape(B, S, D) @ wo

    def _B_ref(x, w_gate, w_up, w_down):
        g = _silu(x @ w_gate)
        u = x @ w_up
        return (g * u) @ w_down

    x = A_x
    xn = _layernorm(x, axis=-1)
    return x + _A_ref(xn, A_wqkv, A_wo) + _B_ref(xn, B_w_gate, B_w_up, B_w_down)
```

```python
import functools
import math
import numpy as np
import jax
import jax.numpy as jnp
from jax import lax
import jax.experimental.pallas as pl
import jax.experimental.pallas.tpu as pltpu

S, D, H, DH, F = 2048, 640, 32, 20, 1536
BQ = 512
BT = 512
NQ = S // BQ
LANE = 128
NG = D // LANE
CROSS = [h for h in range(H) if (DH * h) // LANE != (DH * h + DH - 1) // LANE]
QSCALE = float(DH ** -0.5 * math.log2(math.e))
NT = (((1,), (1,)), ((), ()))
TN = (((0,), (0,)), ((), ()))


def _kernel(x_hbm, wqkv_hbm, wo_hbm, wg_hbm, wu_hbm, wd_hbm, out_hbm,
            x_v, wqkv_v, wo_v, wg_v, wu_v, wd_v,
            xn_v, q_v, k_v, vt_v, at_v, s_v, p_v, m_v, o_v, sems, osems, *, KC, XP):
    nt = S // BT
    x_cp = [pltpu.make_async_copy(x_hbm.at[pl.ds(i * BT, BT)], x_v.at[pl.ds(i * BT, BT)], sems.at[i]) for i in range(nt)]
    w_cp = [pltpu.make_async_copy(a, b, sems.at[nt + i]) for i, (a, b) in enumerate(
        [(wqkv_hbm, wqkv_v), (wg_hbm, wg_v), (wu_hbm, wu_v), (wd_hbm, wd_v), (wo_hbm, wo_v)])]
    x_cp[0].start()
    w_cp[0].start()
    for c in x_cp[1:]:
        c.start()
    for c in w_cp[1:]:
        c.start()

    at_v[...] = jnp.zeros(at_v.shape, at_v.dtype)

    lane = lax.broadcasted_iota(jnp.int32, (BT, LANE), 1)
    for i in range(nt):
        x_cp[i].wait()
        rows = pl.ds(i * BT, BT)
        x = x_v[rows, :].astype(jnp.float32)
        mu = jnp.mean(x, axis=-1, keepdims=True)
        xc = x - mu
        var = jnp.mean(xc * xc, axis=-1, keepdims=True)
        xn = (xc * lax.rsqrt(var + 1e-5)).astype(jnp.bfloat16)
        xn_v[rows, :] = xn
        if i == 0:
            w_cp[0].wait()
        q = jnp.dot(xn, wqkv_v[:, 0:D], preferred_element_type=jnp.float32) * QSCALE
        k = jnp.dot(xn, wqkv_v[:, D:2 * D], preferred_element_type=jnp.float32)
        v = jnp.dot(xn, wqkv_v[:, 2 * D:3 * D], preferred_element_type=jnp.float32)
        for (val, ref) in ((q, q_v), (k, k_v)):
            for g in range(NG):
                ref[g, rows, :] = val[:, g * LANE:(g + 1) * LANE].astype(jnp.bfloat16)
            for j, h in enumerate(CROSS):
                g = (DH * h) // LANE
                ref[NG + j, rows, :] = jnp.where(
                    lane >= (DH * h) % LANE, val[:, g * LANE:(g + 1) * LANE],
                    val[:, (g + 1) * LANE:(g + 2) * LANE]).astype(jnp.bfloat16)
        vt_v[:, rows] = v.T.astype(jnp.bfloat16)

    def head_of(step):
        return step // NQ, step % NQ

    NC = S // KC

    def qk_prep(step):
        h, qb = head_of(step)
        c0 = h * DH
        g0 = c0 // LANE
        g1 = (c0 + DH - 1) // LANE
        g = jnp.where(g0 != g1, NG + g0, g0)
        ln = lax.broadcasted_iota(jnp.int32, (BQ, LANE), 1)
        msk = ((ln - c0) & (LANE - 1)) < DH
        qraw = q_v[g, pl.ds(pl.multiple_of(qb * BQ, BQ), BQ), :]
        qm = jnp.where(msk, qraw.astype(jnp.float32), 0.0)
        if XP:
            qm = qm.astype(jnp.bfloat16)
        else:
            qm = qm.T.astype(jnp.bfloat16)
        return g, qm

    def qk_chunk(g, qm, slot, c, mx):
        kc = k_v[g, c * KC:(c + 1) * KC, :]
        if XP:
            st = lax.dot_general(kc, qm, NT, preferred_element_type=jnp.float32)
        else:
            st = jnp.dot(kc, qm, preferred_element_type=jnp.float32)
        s_v[slot, c * KC:(c + 1) * KC, :] = st
        cm = jnp.max(st.reshape(KC // 8, 8, BQ), axis=0)
        return cm if mx is None else jnp.maximum(mx, cm)

    def step_fn(qstep, qslot, pstep, pslot):
        if qstep is not None:
            g, qm = qk_prep(qstep)
        if pstep is not None:
            h, qb = head_of(pstep)
            c0 = h * DH
            a = pl.multiple_of((c0 // 16) * 16, 16)
            r = c0 - a
            m = jnp.broadcast_to(m_v[pslot], (KC, BQ))
            rw = lax.broadcasted_iota(jnp.int32, (32, KC), 0)
            vmask = (rw >= r) & (rw < r + DH)
        mx = None
        ot = None
        for c in range(NC):
            if qstep is not None:
                mx = qk_chunk(g, qm, qslot, c, mx)
            if pstep is not None:
                p = jnp.exp2(s_v[pslot, c * KC:(c + 1) * KC, :] - m).astype(jnp.bfloat16)
                vt = vt_v[pl.ds(a, 32), c * KC:(c + 1) * KC].astype(jnp.float32)
                vt = jnp.where(vmask, vt, 1.0).astype(jnp.bfloat16)
                d = jnp.dot(vt, p, preferred_element_type=jnp.float32)
                ot = d if ot is None else ot + d
        if qstep is not None:
            m_v[qslot] = jnp.max(mx, axis=0, keepdims=True)
        if pstep is not None:
            l = jnp.where(r == 0, ot[31:32, :], ot[0:1, :])
            rw2 = lax.broadcasted_iota(jnp.int32, (32, BQ), 0)
            cols = pl.ds(pl.multiple_of(qb * BQ, BQ), BQ)
            old = at_v[pl.ds(a, 32), cols]
            at_v[pl.ds(a, 32), cols] = jnp.where((rw2 >= r) & (rw2 < r + DH), ot / l, old)

    nsteps = H * NQ
    step_fn(0, 0, None, None)

    def body(i, c):
        step_fn(2 * i + 1, 1, 2 * i, 0)
        step_fn(jnp.minimum(2 * i + 2, nsteps - 1), 0, 2 * i + 1, 1)
        return c
    lax.fori_loop(0, nsteps // 2, body, 0)

    for c in w_cp[1:]:
        c.wait()

    o_cp = [pltpu.make_async_copy(o_v.at[pl.ds(i * BT, BT)], out_hbm.at[pl.ds(i * BT, BT)], osems.at[i]) for i in range(nt)]
    for i in range(nt):
        rows = pl.ds(i * BT, BT)
        xn = xn_v[rows, :]
        g = jnp.dot(xn, wg_v[...], preferred_element_type=jnp.float32)
        u = jnp.dot(xn, wu_v[...], preferred_element_type=jnp.float32)
        hcur = (g * (1.0 / (1.0 + jnp.exp(-g))) * u).astype(jnp.bfloat16)
        y = jnp.dot(hcur, wd_v[...], preferred_element_type=jnp.float32)
        at = at_v[:, rows].T.astype(jnp.bfloat16)
        y = y + jnp.dot(at, wo_v[...], preferred_element_type=jnp.float32)
        o_v[rows, :] = (x_v[rows, :].astype(jnp.float32) + y).astype(o_v.dtype)
        o_cp[i].start()
    for c in o_cp:
        c.wait()


def make(KC=128, XP=True):
    def f(A_x, A_wqkv, A_wo, B_x, B_w_gate, B_w_up, B_w_down):
        bf = jnp.bfloat16
        x2 = A_x.reshape(S, D)
        nt = S // BT
        out = pl.pallas_call(
            functools.partial(_kernel, KC=KC, XP=XP),
            out_shape=jax.ShapeDtypeStruct((S, D), A_x.dtype),
            in_specs=[pl.BlockSpec(memory_space=pl.ANY)] * 6,
            out_specs=pl.BlockSpec(memory_space=pl.ANY),
            scratch_shapes=[
                pltpu.VMEM((S, D), bf), pltpu.VMEM((D, 3 * D), bf), pltpu.VMEM((D, D), bf),
                pltpu.VMEM((D, F), bf), pltpu.VMEM((D, F), bf), pltpu.VMEM((F, D), bf),
                pltpu.VMEM((S, D), bf),
                pltpu.VMEM((NG + len(CROSS), S, LANE), bf), pltpu.VMEM((NG + len(CROSS), S, LANE), bf),
                pltpu.VMEM((D, S), bf), pltpu.VMEM((D, S), jnp.float32),
                pltpu.VMEM((2, S, BQ), jnp.float32), pltpu.VMEM((S, BQ), bf), pltpu.VMEM((2, 1, BQ), jnp.float32),
                pltpu.VMEM((S, D), bf),
                pltpu.SemaphoreType.DMA((nt + 5,)), pltpu.SemaphoreType.DMA((nt,)),
            ],
            compiler_params=pltpu.CompilerParams(vmem_limit_bytes=110 * 2**20),
        )(x2, A_wqkv, A_wo, B_w_gate, B_w_up, B_w_down)
        return out.reshape(1, S, D)
    return f


@jax.jit
def pallas_parallel_sum__mha_block__swiglu_ffn__prompt_kernel(A_x, A_wqkv, A_wo, B_x, B_w_gate, B_w_up, B_w_down):
    return make()(A_x, A_wqkv, A_wo, B_x, B_w_gate, B_w_up, B_w_down)
```

```python
import math

import jax
import jax.numpy as jnp
import numpy as np
from jax import lax
import jax.experimental.pallas as pl
import jax.experimental.pallas.tpu as pltpu

S, D, H, F = 2048, 640, 32, 1536
DH = D // H
LANE = 128
BQ = 512
KC = 128
NQ, NC, QT, NT, NG = S // BQ, S // KC, BQ // LANE, S // LANE, D // LANE
CROSS = [h for h in range(H) if DH * h // LANE != (DH * h + DH - 1) // LANE]
VR = 24
QR = 32
XB = 512
FB = 256
HB = H * FB // S
UH = 3
OB = (128, 128, 256, 256, 256, 256, 256, 256, 128, 128)

LIVE = (16, 0) * (NC // 2)
EARLY = (0, 16, 0, 16, 0, 16, 0, 0) * (NC // 8)
LIVE_OFF = np.concatenate([[0], np.cumsum(LIVE)]).tolist()
EARLY_OFF = np.concatenate([[0], np.cumsum(EARLY)]).tolist()
N_LIVE, N_EARLY = LIVE_OFF[-1], EARLY_OFF[-1]
LIVE_ROW = [(c + 1) * KC - LIVE[c] + j for c in range(NC) for j in range(0, LIVE[c], 8)]

QSCALE = float(DH ** -0.5 * math.log2(math.e))
F32, BF16, I32 = jnp.float32, jnp.bfloat16, jnp.int32


def _dot(a, b):
    return lax.dot_general(a, b, (((1,), (0,)), ((), ())), preferred_element_type=F32)


def _after(value, other, true):
    if other.dtype != value.dtype:
        other = pltpu.bitcast(other, value.dtype)
    reps = (value.shape[0] // 8, value.shape[1] // LANE)
    if reps != (1, 1):
        true, other = jnp.tile(true, reps), jnp.tile(other, reps)
    return jnp.where(true, value, other)


def _lanes(t):
    return slice(t * LANE, (t + 1) * LANE)


def _cyclic(t, h):
    return jnp.concatenate([t[DH * h:DH * (h + 1)], t[DH * h:DH * h + QR - DH]], axis=0)


def _kernel(x_hbm, wqkv_hbm, wo_hbm, wg_hbm, wu_hbm, wd_hbm, out_hbm,
            x_v, wo_v, k_v, qm_v, qf_v, kb_v, vt_v, es_v, em_v, wqkv_v, wg_v, wu_v, wd_v,
            xn_v, kf_v, kt_v, s0_v, s1_v, m_v, ot_v, xsems, wsems, osems):
    x_cp = [pltpu.make_async_copy(x_hbm.at[pl.ds(i * XB, XB)], x_v.at[pl.ds(i * XB, XB)], xsems.at[i])
            for i in range(S // XB)]
    wq_cp, wk_cp, wv_cp = [
        pltpu.make_async_copy(wqkv_hbm.at[:, pl.ds(i * D, D)], wqkv_v.at[i], wsems.at[i]) for i in range(3)]
    w_cp = [pltpu.make_async_copy(src, dst, wsems.at[3 + i]) for i, (src, dst) in enumerate(
        [(wg_hbm, wg_v), (wu_hbm, wu_v), (wd_hbm, wd_v), (wo_hbm, wo_v)])]

    def layernorm(lo, marks=(), true=None):
        n = 16 if marks else XB
        for j in range(XB // n):
            r = lo + n * j
            x = x_v[pl.ds(r, n), :]
            if marks:
                mark = marks[j * len(marks) // (XB // n)]
                x = pltpu.bitcast(_after(pltpu.bitcast(x, I32), mark, true), BF16)
            x = x.astype(F32)
            xc = x - jnp.mean(x, axis=-1, keepdims=True)
            var = jnp.mean(xc * xc, axis=-1, keepdims=True)
            xn_v[pl.ds(r // 2, n // 2), :] = pltpu.bitcast((xc * lax.rsqrt(var + 1e-5)).astype(BF16), I32)

    def project(which, lo, n, quartered):
        xn = pltpu.bitcast(xn_v[pl.ds(lo // 2, n // 2), :], BF16)
        if quartered:
            val = jnp.concatenate([
                _dot(xn, wqkv_v[which, :, 0:4 * LANE]),
                jnp.concatenate([_dot(xn[j * n // 4:(j + 1) * n // 4], wqkv_v[which, :, 4 * LANE:D])
                                 for j in range(4)], axis=0)], axis=1)
        else:
            val = _dot(xn, wqkv_v[which])
        return val, [val[r:r + 8, _lanes(g)] for g in range(NG) for r in range(0, n, 128)]

    def project_q(lo):
        val, marks = project(0, lo, XB, False)
        cols = pl.ds(lo, XB)
        qt = (val * QSCALE).T
        q32 = pltpu.bitcast(qt.astype(BF16), I32)
        row = lax.broadcasted_iota(I32, (8, XB), 0)
        for h in range(H):
            first = DH // 2 * h
            v = first // 8
            qm_v[h, pl.ds(v % 8 * 8, 8), cols] = jnp.where(row >= first - 8 * v, q32[8 * v:8 * v + 8], 0)
            v += 1
            qm_v[h, pl.ds(v % 8 * 8, 8), cols] = jnp.where(
                row < first + DH // 2 - 8 * v, q32[8 * v:8 * v + 8], 0)
            ext = _cyclic(qt, h)
            for t in range(XB // LANE):
                qf_v[lo // LANE + t, QR * h:QR * (h + 1), :] = ext[:, _lanes(t)]
        return marks

    def project_k(lo, quartered=False):
        val, marks = project(1, lo, XB, quartered)
        half = pl.ds(lo // 2, XB // 2)
        lane = lax.broadcasted_iota(I32, (XB, LANE), 1)
        for g in range(NG):
            k_v[g, half, :] = pltpu.bitcast(val[:, _lanes(g)].astype(BF16), I32)
        for j, h in enumerate(CROSS):
            g = DH * h // LANE
            mix = jnp.where(lane >= DH * h % LANE, val[:, _lanes(g)], val[:, _lanes(g + 1)])
            k_v[NG + j, half, :] = pltpu.bitcast(mix.astype(BF16), I32)
        for c in range(lo // KC, (lo + XB) // KC):
            end = (c + 1) * KC - lo
            if LIVE[c]:
                kf_v[0, LIVE_OFF[c]:LIVE_OFF[c + 1], :] = val[end - LIVE[c]:end, :]
            if EARLY[c]:
                kf_v[1, EARLY_OFF[c]:EARLY_OFF[c + 1], :] = val[end - EARLY[c]:end, :]
        return marks

    def project_v(lo, n=XB, quartered=False):
        val, marks = project(2, lo, n, quartered)
        vt = val.T
        row = lax.broadcasted_iota(I32, (VR, n), 0)
        for h in range(H):
            a = DH * h // 8 * 8
            r = DH * h - a
            vt_v[h, :, pl.ds(lo, n)] = jnp.where((row >= r) & (row < r + DH), vt[a:a + VR], 1.0)
        return marks

    def skew_keys(marks, true):
        sub = lax.broadcasted_iota(I32, (VR, LANE), 1) & 7
        for j in (1, 0):
            kt = kf_v[j].T
            for h in range(H):
                ext = _after(_cyclic(kt, h), marks[((1 - j) * H + h) * len(marks) // (2 * H)], true)
                sk = ext[0:VR]
                for s in range(1, 8):
                    sk = jnp.where(sub == s, ext[s:s + VR], sk)
                kt_v[j, h] = sk

    def splat_keys(j, h, i):
        return jnp.broadcast_to(kt_v[j, h, i:i + 1, :], (LANE, LANE)).T

    def staged(j, i, e, zero=0):
        v = (j * DH + i) * (N_EARLY // 8) + e
        row = (v // QT + zero) * 8
        return pl.ds(row if isinstance(row, int) else pl.multiple_of(row, 8), 8), pl.ds(v % QT * LANE, LANE)

    def stage_keys(dst_v, j, h):
        for i in range(DH):
            kb = splat_keys(1, h, i)
            for e in range(N_EARLY // 8):
                dst_v[staged(j, i, e)] = kb[e * 8:(e + 1) * 8]

    x_cp[0].start()
    wk_cp.start()
    for h in range(H):
        for j in range(2, 8):
            qm_v[h, pl.ds((DH // 2 * h // 8 + j) % 8 * 8, 8), :] = jnp.zeros((8, S), I32)
    kf_v[1, N_EARLY:, :] = jnp.zeros((LANE - N_EARLY, D), F32)
    x_cp[0].wait()
    wv_cp.start()
    layernorm(0)
    wk_cp.wait()
    x_cp[1].start()
    wq_cp.start()
    project_k(0, quartered=True)
    wv_cp.wait()
    x_cp[1].wait()
    for cp in x_cp[2:]:
        cp.start()
    true = (pltpu.bitcast(x_v[0:16, 0:LANE], I32) & 1) < 2
    layernorm(XB, project_v(0)[:14], true)
    project_k(XB)
    project_v(XB, quartered=True)
    wq_cp.wait()
    for cp in x_cp[2:]:
        cp.wait()
    for cp in w_cp:
        cp.start()
    layernorm(2 * XB, (project_q(0) + project_q(XB))[:32], true)
    layernorm(3 * XB, (project_k(2 * XB) + project_v(2 * XB))[:32], true)
    project_k(3 * XB)
    skew_keys(project_q(2 * XB) + project_q(3 * XB), true)
    for j in range(HB):
        stage_keys(s0_v, j, j)
    project_v(3 * XB, XB - LANE)
    project_v(S - LANE, LANE)
    for cp in w_cp:
        cp.wait()

    def swiglu(blk, cur_v, nxt_v, zero):
        true = lax.broadcasted_iota(I32, (8, LANE), 0) >= -blk
        rows = pl.ds(pl.multiple_of(blk * FB, FB), FB)
        for j in range(HB):
            h = blk * HB + j
            stage_keys(nxt_v, j, jnp.minimum(h + HB, H - 1))
            for i in range(DH):
                kb_v[h * DH + i] = splat_keys(0, h, i)

        def early_scores():
            for j in range(HB):
                h = blk * HB + j
                for t0 in range(0, NT, 2):
                    top = {}
                    for e0 in range(0, N_EARLY // 8, 3):
                        acc = {}
                        for i in range(DH):
                            kb = {e: cur_v[staged(j, i, e, zero)] for e in range(e0, e0 + 3)}
                            for t in (t0, t0 + 1):
                                q = qf_v[t, pl.ds(h * QR + i, 8), :]
                                for e in kb:
                                    acc[e, t] = kb[e] * q if i == 0 else acc[e, t] + kb[e] * q
                                    yield acc[e, t]
                        for (e, t), s in acc.items():
                            es_v[h, e * 8:(e + 1) * 8, _lanes(t)] = s
                            top[t] = jnp.maximum(top[t], s) if t in top else s
                    for t, s in top.items():
                        em_v[h, :, _lanes(t)] = jnp.max(s, axis=0, keepdims=True)

        side = early_scores()
        n_side = HB * N_EARLY // 8 * NT * DH
        n_slots = 3 * D * F // (4 * LANE * LANE) * FB // 16
        seen = dict(tile=0, slot=0, side=0)

        def paced_dot(a32, w):
            cols = []
            for g in range(a32.shape[1] // LANE):
                col = a32[:, _lanes(g)]
                if seen["tile"] % 4 == 0:
                    parts = []
                    for r in range(FB // 16):
                        seen["slot"] += 1
                        while seen["side"] < n_side * seen["slot"] // n_slots:
                            done = next(side)
                            seen["side"] += 1
                        parts.append(_after(col[r * 8:(r + 1) * 8], done, true))
                    col = jnp.concatenate(parts, axis=0)
                seen["tile"] += 1
                cols.append(col)
            return _dot(pltpu.bitcast(jnp.concatenate(cols, axis=1), BF16), w)

        xn = xn_v[pl.ds(pl.multiple_of(blk * (FB // 2), FB // 2), FB // 2), :]
        hidden = []
        for n in range(F // LANE):
            g = 0.5 * paced_dot(xn, wg_v[:, _lanes(n)])
            u = paced_dot(xn, wu_v[:, _lanes(n)])
            hidden.append(pltpu.bitcast(((g * jnp.tanh(g) + g) * u).astype(BF16), I32))
        hidden = jnp.concatenate(hidden, axis=1)
        x = x_v[rows, :]
        y = [(x[:, _lanes(n)].astype(F32) + paced_dot(hidden, wd_v[:, _lanes(n)])).astype(BF16)
             for n in range(NG)]
        for _ in side:
            pass
        x_v[rows, :] = jnp.concatenate(y, axis=1)

    def swiglu_pair(i, carry):
        swiglu(2 * i, s0_v, s1_v, 0)
        swiglu(2 * i + 1, s1_v, s0_v, i >> 16)
        return carry

    lax.fori_loop(0, S // FB // 2, swiglu_pair, 0)

    s_v = (s0_v, s1_v)

    def key_group(h):
        g0, g1 = h * DH // LANE, (h * DH + DH - 1) // LANE
        if isinstance(h, int):
            return g0 if g0 == g1 else NG + g0
        return jnp.where(g0 != g1, NG + g0, g0)

    def weigh_values(h, qb, c):
        cols = pl.ds(qb * BQ, BQ)
        s = s_v[qb % 2][pl.ds(c * KC, KC - EARLY[c]), :]
        if EARLY[c]:
            s = jnp.concatenate([s, es_v[h, EARLY_OFF[c]:EARLY_OFF[c + 1], cols]], axis=0)
        p = jnp.exp2(s.reshape(KC // 8, 8, BQ) - m_v[qb % 2][None]).reshape(KC, BQ).astype(BF16)
        ot = _dot(vt_v[h, :, pl.ds(c * KC, KC)], p)
        if c > 0:
            ot = ot_v[...] + ot
        if c < NC - 1:
            ot_v[...] = ot
        else:
            es_v[h, 0:VR, cols] = ot

    def step(h, qb, true, marks):
        cols = pl.ds(qb * BQ, BQ)
        g = key_group(h)
        top, top_live = [None] * QT, [None] * QT

        def raise_to(m, t, s):
            m[t] = s if m[t] is None else jnp.maximum(m[t], s)

        def live_scores():
            for e0 in range(0, N_LIVE // 8, 2):
                for t0 in range(0, QT, 2):
                    acc = {}
                    for i in range(DH):
                        kb = {e: kb_v[h * DH + i, e * 8:(e + 1) * 8, :] for e in (e0, e0 + 1)}
                        for t in (t0, t0 + 1):
                            q = qf_v[qb * QT + t, pl.ds(h * QR + i, 8), :]
                            if i == 0 and len(marks) >= 5:
                                q = _after(q, marks[-5], true)
                            for e in kb:
                                acc[e, t] = kb[e] * q if i == 0 else acc[e, t] + kb[e] * q
                                yield acc[e, t]
                    for (e, t), s in acc.items():
                        s_v[qb % 2][pl.ds(LIVE_ROW[e], 8), _lanes(t)] = s
                        raise_to(top_live, t, s)

        side = live_scores()
        n_side = N_LIVE // 8 * QT * DH
        n_slots = (S - N_LIVE - N_EARLY) // 8 + 4 * NC
        issued = slot = 0
        for c in range(NC):
            n = KC - LIVE[c] - EARLY[c]
            k32 = k_v[g, pl.ds(c * KC // 2, n // 2), :]
            parts = []
            for r in range(n // 16):
                slot += 6 if r == 4 else 2
                while issued < n_side * slot // n_slots:
                    done = next(side)
                    issued += 1
                parts.append(_after(k32[r * 8:(r + 1) * 8], done, true))
            st = _dot(pltpu.bitcast(jnp.concatenate(parts, axis=0), BF16), pltpu.bitcast(qm_v[h, :, cols], BF16))
            s_v[qb % 2][pl.ds(c * KC, n), :] = st
            marks += [st[0:8, 0:LANE], st[64:72, 0:LANE]]
            for r in range(n // 8):
                for t in range(QT):
                    raise_to(top, t, st[r * 8:(r + 1) * 8, _lanes(t)])
            back = 1 if c > 0 else 2
            if qb >= back:
                weigh_values(h, qb - back, (c - 1) % NC)
            elif not (isinstance(h, int) and h == 0):
                weigh_values(h - 1, qb - back + NQ, (c - 1) % NC)
        for _ in side:
            pass
        for t in range(QT):
            raise_to(top, t, top_live[t])
        m = jnp.max(jnp.concatenate(top, axis=1), axis=0, keepdims=True)
        m_v[qb % 2] = jnp.broadcast_to(jnp.maximum(m, em_v[h, :, cols]), (8, BQ))

    def heads(h0, count, true):
        marks = []
        for u in range(count):
            for qb in range(NQ):
                step(h0 + u, qb, true, marks)

    def heads_body(i, carry):
        heads(1 + i * UH, UH, lax.broadcasted_iota(I32, (8, LANE), 0) >= -i)
        return carry

    heads(0, 1, qm_v[0, 16:24, 0:LANE] == 0)
    lax.fori_loop(0, (H - 2) // UH, heads_body, 0)
    true = qm_v[0, 16:24, 0:LANE] == 0
    heads(H - 1, 1, true)

    start = np.concatenate([[0], np.cumsum(OB)]).tolist()
    o_cp = [pltpu.make_async_copy(x_v.at[pl.ds(start[i], n)], out_hbm.at[pl.ds(start[i], n)], osems.at[i])
            for i, n in enumerate(OB)]
    tail = [(NQ - 2, NC - 1)] + [(NQ - 1, c) for c in range(NC)]
    n_ready = len([end for end in start[1:] if end <= (NQ - 2) * BQ])
    mark = None
    for i, n in enumerate(OB):
        rows = pl.ds(start[i], n)
        low = lax.broadcasted_iota(I32, (8, n), 0) < 4
        parts = []
        for h in range(0, H, 2):
            a, b = es_v[h, 0:VR, rows], es_v[h + 1, 0:VR, rows]
            den = jnp.where(low, b[0:8], a[16:24])
            if mark is not None:
                den = _after(den, mark, true)
            inv = 1.0 / den
            ia, ib = jnp.broadcast_to(inv[7:8], (8, n)), jnp.broadcast_to(inv[0:1], (8, n))
            parts += [a[0:8] * ia, a[8:16] * ia, jnp.where(low, a[16:24] * ia, b[0:8] * ib),
                      b[8:16] * ib, b[16:24] * ib]
        res = _dot(jnp.concatenate(parts, axis=0).T.astype(BF16), wo_v[...])
        mark = res[0:8, 0:LANE]
        x_v[rows, :] = (x_v[rows, :].astype(F32) + res).astype(BF16)
        o_cp[i].start()
        if i < n_ready:
            for qb, c in tail[i * len(tail) // n_ready:(i + 1) * len(tail) // n_ready]:
                weigh_values(H - 1, qb, c)
    for cp in o_cp:
        cp.wait()


@jax.jit
def pallas_parallel_sum__mha_block__swiglu_ffn__prompt_kernel(
    A_x: jax.Array,
    A_wqkv: jax.Array,
    A_wo: jax.Array,
    B_x: jax.Array,
    B_w_gate: jax.Array,
    B_w_up: jax.Array,
    B_w_down: jax.Array,
):
    del B_x
    out = pl.pallas_call(
        _kernel,
        out_shape=jax.ShapeDtypeStruct((S, D), A_x.dtype),
        in_specs=[pl.BlockSpec(memory_space=pl.ANY)] * 6,
        out_specs=pl.BlockSpec(memory_space=pl.ANY),
        scratch_shapes=[
            pltpu.VMEM((S, D), BF16),
            pltpu.VMEM((D, D), BF16),
            pltpu.VMEM((NG + len(CROSS), S // 2, LANE), I32),
            pltpu.VMEM((H, LANE // 2, S), I32),
            pltpu.VMEM((NT, H * QR, LANE), F32),
            pltpu.VMEM((D, LANE, LANE), F32),
            pltpu.VMEM((H, VR, S), F32),
            pltpu.VMEM((H, N_EARLY, S), F32),
            pltpu.VMEM((H, 1, S), F32),
            pltpu.VMEM((3, D, D), BF16),
            pltpu.VMEM((D, F), BF16),
            pltpu.VMEM((D, F), BF16),
            pltpu.VMEM((F, D), BF16),
            pltpu.VMEM((S // 2, D), I32),
            pltpu.VMEM((2, LANE, D), F32),
            pltpu.VMEM((2, H, VR, LANE), F32),
            pltpu.VMEM((S, BQ), F32),
            pltpu.VMEM((S, BQ), F32),
            pltpu.VMEM((2, 8, BQ), F32),
            pltpu.VMEM((VR, BQ), F32),
            pltpu.SemaphoreType.DMA((S // XB,)),
            pltpu.SemaphoreType.DMA((7,)),
            pltpu.SemaphoreType.DMA((len(OB),)),
        ],
        compiler_params=pltpu.CompilerParams(vmem_limit_bytes=127 * 2**20),
    )(A_x.reshape(S, D), A_wqkv, A_wo, B_w_gate, B_w_up, B_w_down)
    return out.reshape(A_x.shape)
```

```python
import math

import jax
import jax.numpy as jnp
import numpy as np
from jax import lax
import jax.experimental.pallas as pl
import jax.experimental.pallas.tpu as pltpu

S, D, H, F = 2048, 640, 32, 1536
DH = D // H
LANE = 128
BQ = 512
KC = 128
NQ, NC, QT, NT, NG = S // BQ, S // KC, BQ // LANE, S // LANE, D // LANE
CROSS = [h for h in range(H) if DH * h // LANE != (DH * h + DH - 1) // LANE]
VR = 24
QR = 32
XB = 512
FB = 256
HB = H * FB // S
UH = 3
OB = (128, 128, 256, 256, 256, 256, 256, 256, 128, 128)

LIVE = (16, 0) * (NC // 2)
EARLY = (0, 16, 0, 16, 0, 16, 0, 0) * (NC // 8)
LIVE_OFF = np.concatenate([[0], np.cumsum(LIVE)]).tolist()
EARLY_OFF = np.concatenate([[0], np.cumsum(EARLY)]).tolist()
N_LIVE, N_EARLY = LIVE_OFF[-1], EARLY_OFF[-1]
LIVE_ROW = [(c + 1) * KC - LIVE[c] + j for c in range(NC) for j in range(0, LIVE[c], 8)]

QSCALE = float(DH ** -0.5 * math.log2(math.e))
F32, BF16, I32 = jnp.float32, jnp.bfloat16, jnp.int32


def _dot(a, b):
    return lax.dot_general(a, b, (((1,), (0,)), ((), ())), preferred_element_type=F32)


def _after(value, other, true):
    if other.dtype != value.dtype:
        other = pltpu.bitcast(other, value.dtype)
    reps = (value.shape[0] // 8, value.shape[1] // LANE)
    if reps != (1, 1):
        true, other = jnp.tile(true, reps), jnp.tile(other, reps)
    return jnp.where(true, value, other)


def _outer(k, q):
    return k.reshape(1, k.shape[0] // 8, 8, LANE) * q[:, None]


def _lanes(t):
    return slice(t * LANE, (t + 1) * LANE)


def _cyclic(t, h):
    return jnp.concatenate([t[DH * h:DH * (h + 1)], t[DH * h:DH * h + QR - DH]], axis=0)


def _kernel(x_hbm, wqkv_hbm, wo_hbm, wg_hbm, wu_hbm, wd_hbm, out_hbm,
            x_v, wo_v, k_v, qm_v, qf_v, kb_v, vt_v, es_v, em_v, wqkv_v, wg_v, wu_v, wd_v,
            xn_v, kf_v, kt_v, s0_v, s1_v, m_v, ot_v, xsems, wsems, osems):
    x_cp = [pltpu.make_async_copy(x_hbm.at[pl.ds(i * XB, XB)], x_v.at[pl.ds(i * XB, XB)], xsems.at[i])
            for i in range(S // XB)]
    wq_cp, wk_cp, wv_cp = [
        pltpu.make_async_copy(wqkv_hbm.at[:, pl.ds(i * D, D)], wqkv_v.at[i], wsems.at[i]) for i in range(3)]
    w_cp = [pltpu.make_async_copy(src, dst, wsems.at[3 + i]) for i, (src, dst) in enumerate(
        [(wg_hbm, wg_v), (wu_hbm, wu_v), (wd_hbm, wd_v), (wo_hbm, wo_v)])]

    def layernorm(lo, marks=(), true=None):
        n = 16 if marks else XB
        for j in range(XB // n):
            r = lo + n * j
            x = x_v[pl.ds(r, n), :]
            if marks:
                mark = marks[j * len(marks) // (XB // n)]
                x = pltpu.bitcast(_after(pltpu.bitcast(x, I32), mark, true), BF16)
            x = x.astype(F32)
            xc = x - jnp.mean(x, axis=-1, keepdims=True)
            var = jnp.mean(xc * xc, axis=-1, keepdims=True)
            xn_v[pl.ds(r // 2, n // 2), :] = pltpu.bitcast((xc * lax.rsqrt(var + 1e-5)).astype(BF16), I32)

    def project(which, lo, n, quartered):
        xn = pltpu.bitcast(xn_v[pl.ds(lo // 2, n // 2), :], BF16)
        if quartered:
            val = jnp.concatenate([
                _dot(xn, wqkv_v[which, :, 0:4 * LANE]),
                jnp.concatenate([_dot(xn[j * n // 4:(j + 1) * n // 4], wqkv_v[which, :, 4 * LANE:D])
                                 for j in range(4)], axis=0)], axis=1)
        else:
            val = _dot(xn, wqkv_v[which])
        return val, [val[r:r + 8, _lanes(g)] for g in range(NG) for r in range(0, n, 128)]

    def project_q(lo):
        val, marks = project(0, lo, XB, False)
        cols = pl.ds(lo, XB)
        qt = (val * QSCALE).T
        q32 = pltpu.bitcast(qt.astype(BF16), I32)
        row = lax.broadcasted_iota(I32, (8, XB), 0)
        for h in range(H):
            first = DH // 2 * h
            v = first // 8
            qm_v[h, pl.ds(v % 8 * 8, 8), cols] = jnp.where(row >= first - 8 * v, q32[8 * v:8 * v + 8], 0)
            v += 1
            qm_v[h, pl.ds(v % 8 * 8, 8), cols] = jnp.where(
                row < first + DH // 2 - 8 * v, q32[8 * v:8 * v + 8], 0)
            ext = _cyclic(qt, h)
            for t in range(XB // LANE):
                qf_v[lo // LANE + t, QR * h:QR * (h + 1), :] = ext[:, _lanes(t)]
        return marks

    def project_k(lo, quartered=False):
        val, marks = project(1, lo, XB, quartered)
        half = pl.ds(lo // 2, XB // 2)
        lane = lax.broadcasted_iota(I32, (XB, LANE), 1)
        for g in range(NG):
            k_v[g, half, :] = pltpu.bitcast(val[:, _lanes(g)].astype(BF16), I32)
        for j, h in enumerate(CROSS):
            g = DH * h // LANE
            mix = jnp.where(lane >= DH * h % LANE, val[:, _lanes(g)], val[:, _lanes(g + 1)])
            k_v[NG + j, half, :] = pltpu.bitcast(mix.astype(BF16), I32)
        for c in range(lo // KC, (lo + XB) // KC):
            end = (c + 1) * KC - lo
            if LIVE[c]:
                kf_v[0, LIVE_OFF[c]:LIVE_OFF[c + 1], :] = val[end - LIVE[c]:end, :]
            if EARLY[c]:
                kf_v[1, EARLY_OFF[c]:EARLY_OFF[c + 1], :] = val[end - EARLY[c]:end, :]
        return marks

    def project_v(lo, n=XB, quartered=False):
        val, marks = project(2, lo, n, quartered)
        vt = val.T
        row = lax.broadcasted_iota(I32, (VR, n), 0)
        for h in range(H):
            a = DH * h // 8 * 8
            r = DH * h - a
            vt_v[h, :, pl.ds(lo, n)] = jnp.where((row >= r) & (row < r + DH), vt[a:a + VR], 1.0)
        return marks

    def skew_keys(marks, true):
        sub = lax.broadcasted_iota(I32, (VR, LANE), 1) & 7
        for j in (1, 0):
            kt = kf_v[j].T
            for h in range(H):
                ext = _after(_cyclic(kt, h), marks[((1 - j) * H + h) * len(marks) // (2 * H)], true)
                sk = ext[0:VR]
                for s in range(1, 8):
                    sk = jnp.where(sub == s, ext[s:s + VR], sk)
                kt_v[j, h] = sk

    def splat_keys(j, h, i):
        return jnp.broadcast_to(kt_v[j, h, i:i + 1, :], (LANE, LANE)).T

    def staged(j, i, first, n, zero=0):
        row = (i * N_EARLY + first) + zero * 8
        return j, pl.ds(row if isinstance(row, int) else pl.multiple_of(row, 8), n)

    def stage_keys(dst_v, j, h):
        for i in range(DH):
            dst_v[staged(j, i, 0, N_EARLY)] = splat_keys(1, h, i)[0:N_EARLY]

    x_cp[0].start()
    wk_cp.start()
    for h in range(H):
        for j in range(2, 8):
            qm_v[h, pl.ds((DH // 2 * h // 8 + j) % 8 * 8, 8), :] = jnp.zeros((8, S), I32)
    kf_v[1, N_EARLY:, :] = jnp.zeros((LANE - N_EARLY, D), F32)
    x_cp[0].wait()
    wv_cp.start()
    layernorm(0)
    wk_cp.wait()
    x_cp[1].start()
    project_k(0, quartered=True)
    wv_cp.wait()
    x_cp[1].wait()
    wq_cp.start()
    for cp in x_cp[2:]:
        cp.start()
    true = (pltpu.bitcast(x_v[0:16, 0:LANE], I32) & 1) < 2
    layernorm(XB, project_v(0)[:14], true)
    project_k(XB)
    project_v(XB, quartered=True)
    wq_cp.wait()
    for cp in x_cp[2:]:
        cp.wait()
    for cp in w_cp:
        cp.start()
    layernorm(2 * XB, (project_q(0) + project_q(XB))[:32], true)
    layernorm(3 * XB, (project_k(2 * XB) + project_v(2 * XB))[:32], true)
    project_k(3 * XB)
    skew_keys(project_q(2 * XB) + project_q(3 * XB), true)
    for j in range(HB):
        stage_keys(s0_v, j, j)
    project_v(3 * XB, XB - LANE)
    project_v(S - LANE, LANE)
    for cp in w_cp:
        cp.wait()

    def swiglu(blk, cur_v, nxt_v, zero):
        true = lax.broadcasted_iota(I32, (8, LANE), 0) >= -blk
        rows = pl.ds(pl.multiple_of(blk * FB, FB), FB)
        for j in range(HB):
            h = blk * HB + j
            stage_keys(nxt_v, j, jnp.minimum(h + HB, H - 1))
            for i in range(DH):
                kb_v[h * DH + i] = splat_keys(0, h, i)

        def early_scores():
            for j in range(HB):
                h = blk * HB + j
                for t in range(0, NT, 2):
                    top = None
                    for e in range(0, N_EARLY, 24):
                        for i in range(DH):
                            k = cur_v[staged(j, i, e, 24, zero)]
                            term = _outer(k, qf_v[t:t + 2, pl.ds(h * QR + i, 8), :])
                            acc = term if i == 0 else acc + term
                            yield acc
                        for u in range(2):
                            es_v[h, e:e + 24, _lanes(t + u)] = acc[u].reshape(24, LANE)
                        best = jnp.max(acc, axis=1)
                        top = best if top is None else jnp.maximum(top, best)
                    for u in range(2):
                        em_v[h, :, _lanes(t + u)] = jnp.max(top[u], axis=0, keepdims=True)

        side = early_scores()
        n_side = HB * N_EARLY // 24 * NT // 2 * DH
        n_slots = 3 * D * F // (4 * LANE * LANE) * FB // 16
        seen = dict(tile=0, slot=0, side=0)

        def paced_dot(a32, w):
            cols = []
            for g in range(a32.shape[1] // LANE):
                col = a32[:, _lanes(g)]
                if seen["tile"] % 4 == 0:
                    parts = []
                    for r in range(FB // 16):
                        seen["slot"] += 1
                        while seen["side"] < n_side * seen["slot"] // n_slots:
                            done = next(side)
                            seen["side"] += 1
                        parts.append(_after(col[r * 8:(r + 1) * 8], done[-1, -1], true))
                    col = jnp.concatenate(parts, axis=0)
                seen["tile"] += 1
                cols.append(col)
            return _dot(pltpu.bitcast(jnp.concatenate(cols, axis=1), BF16), w)

        xn = xn_v[pl.ds(pl.multiple_of(blk * (FB // 2), FB // 2), FB // 2), :]
        hidden = []
        for n in range(F // LANE):
            g = 0.5 * paced_dot(xn, wg_v[:, _lanes(n)])
            u = paced_dot(xn, wu_v[:, _lanes(n)])
            hidden.append(pltpu.bitcast(((g * jnp.tanh(g) + g) * u).astype(BF16), I32))
        hidden = jnp.concatenate(hidden, axis=1)
        x = x_v[rows, :]
        y = [(x[:, _lanes(n)].astype(F32) + paced_dot(hidden, wd_v[:, _lanes(n)])).astype(BF16)
             for n in range(NG)]
        for _ in side:
            pass
        x_v[rows, :] = jnp.concatenate(y, axis=1)

    def swiglu_pair(i, carry):
        swiglu(2 * i, s0_v, s1_v, 0)
        swiglu(2 * i + 1, s1_v, s0_v, i >> 16)
        return carry

    lax.fori_loop(0, S // FB // 2, swiglu_pair, 0)

    s_v = (s0_v, s1_v)

    def key_group(h):
        g0, g1 = h * DH // LANE, (h * DH + DH - 1) // LANE
        if isinstance(h, int):
            return g0 if g0 == g1 else NG + g0
        return jnp.where(g0 != g1, NG + g0, g0)

    def weigh_values(h, qb, c):
        cols = pl.ds(qb * BQ, BQ)
        s = jnp.concatenate([s_v[qb % 2][t, pl.ds(c * KC, KC - EARLY[c]), :] for t in range(QT)], axis=1)
        if EARLY[c]:
            s = jnp.concatenate([s, es_v[h, EARLY_OFF[c]:EARLY_OFF[c + 1], cols]], axis=0)
        p = jnp.exp2(s.reshape(KC // 8, 8, BQ) - m_v[qb % 2][None]).reshape(KC, BQ).astype(BF16)
        ot = _dot(vt_v[h, :, pl.ds(c * KC, KC)], p)
        if c > 0:
            ot = ot_v[...] + ot
        if c < NC - 1:
            ot_v[...] = ot
        else:
            es_v[h, 0:VR, cols] = ot

    def step(h, qb, true, marks):
        cols = pl.ds(qb * BQ, BQ)
        g = key_group(h)
        top_live = {}

        def live_scores():
            for e in range(0, N_LIVE, 16):
                for t in range(0, QT, 2):
                    for i in range(DH):
                        q = qf_v[qb * QT + t:qb * QT + t + 2, pl.ds(h * QR + i, 8), :]
                        if i == 0 and len(marks) >= 5:
                            q = jnp.where(true[None], q, marks[-5][None])
                        term = _outer(kb_v[h * DH + i, e:e + 16, :], q)
                        acc = term if i == 0 else acc + term
                        yield acc
                    s_v[qb % 2][t:t + 2, pl.ds(LIVE_ROW[e // 8], 16), :] = acc.reshape(2, 16, LANE)
                    best = jnp.max(acc, axis=1)
                    top_live[t] = jnp.maximum(top_live[t], best) if t in top_live else best

        side = live_scores()
        n_side = N_LIVE // 16 * QT // 2 * DH
        n_slots = (S - N_LIVE - N_EARLY) // 8 + 4 * NC
        issued = slot = 0
        for c in range(NC):
            n = KC - LIVE[c] - EARLY[c]
            k32 = k_v[g, pl.ds(c * KC // 2, n // 2), :]
            parts = []
            for r in range(n // 16):
                slot += 6 if r == 4 else 2
                while issued < n_side * slot // n_slots:
                    done = next(side)
                    issued += 1
                parts.append(_after(k32[r * 8:(r + 1) * 8], done[-1, -1], true))
            st = _dot(pltpu.bitcast(jnp.concatenate(parts, axis=0), BF16), pltpu.bitcast(qm_v[h, :, cols], BF16))
            for t in range(QT):
                s_v[qb % 2][t, pl.ds(c * KC, n), :] = st[:, _lanes(t)]
            marks += [st[0:8, 0:LANE], st[64:72, 0:LANE]]
            best = jnp.max(st.reshape(n // 8, 8, BQ), axis=0)
            top = best if c == 0 else jnp.maximum(top, best)
            back = 1 if c > 0 else 2
            if qb >= back:
                weigh_values(h, qb - back, (c - 1) % NC)
            elif not (isinstance(h, int) and h == 0):
                weigh_values(h - 1, qb - back + NQ, (c - 1) % NC)
        for _ in side:
            pass
        top = jnp.maximum(top, jnp.concatenate([top_live[t - t % 2][t % 2] for t in range(QT)], axis=1))
        m = jnp.max(top, axis=0, keepdims=True)
        m_v[qb % 2] = jnp.broadcast_to(jnp.maximum(m, em_v[h, :, cols]), (8, BQ))

    def heads(h0, count, true):
        marks = []
        for u in range(count):
            for qb in range(NQ):
                step(h0 + u, qb, true, marks)

    def heads_body(i, carry):
        heads(1 + i * UH, UH, lax.broadcasted_iota(I32, (8, LANE), 0) >= -i)
        return carry

    heads(0, 1, qm_v[0, 16:24, 0:LANE] == 0)
    lax.fori_loop(0, (H - 2) // UH, heads_body, 0)
    true = qm_v[0, 16:24, 0:LANE] == 0
    heads(H - 1, 1, true)

    start = np.concatenate([[0], np.cumsum(OB)]).tolist()
    o_cp = [pltpu.make_async_copy(x_v.at[pl.ds(start[i], n)], out_hbm.at[pl.ds(start[i], n)], osems.at[i])
            for i, n in enumerate(OB)]
    tail = [(NQ - 2, NC - 1)] + [(NQ - 1, c) for c in range(NC)]
    n_ready = len([end for end in start[1:] if end <= (NQ - 2) * BQ])
    mark = None
    for i, n in enumerate(OB):
        rows = pl.ds(start[i], n)
        low = lax.broadcasted_iota(I32, (8, n), 0) < 4
        parts = []
        for h in range(0, H, 2):
            a, b = es_v[h, 0:VR, rows], es_v[h + 1, 0:VR, rows]
            den = jnp.where(low, b[0:8], a[16:24])
            if mark is not None:
                den = _after(den, mark, true)
            inv = 1.0 / den
            ia, ib = jnp.broadcast_to(inv[7:8], (8, n)), jnp.broadcast_to(inv[0:1], (8, n))
            parts += [a[0:8] * ia, a[8:16] * ia, jnp.where(low, a[16:24] * ia, b[0:8] * ib),
                      b[8:16] * ib, b[16:24] * ib]
        res = _dot(jnp.concatenate(parts, axis=0).T.astype(BF16), wo_v[...])
        mark = res[0:8, 0:LANE]
        x_v[rows, :] = (x_v[rows, :].astype(F32) + res).astype(BF16)
        o_cp[i].start()
        if i < n_ready:
            for qb, c in tail[i * len(tail) // n_ready:(i + 1) * len(tail) // n_ready]:
                weigh_values(H - 1, qb, c)
    for cp in o_cp:
        cp.wait()


@jax.jit
def pallas_parallel_sum__mha_block__swiglu_ffn__prompt_kernel(
    A_x: jax.Array,
    A_wqkv: jax.Array,
    A_wo: jax.Array,
    B_x: jax.Array,
    B_w_gate: jax.Array,
    B_w_up: jax.Array,
    B_w_down: jax.Array,
):
    del B_x
    out = pl.pallas_call(
        _kernel,
        out_shape=jax.ShapeDtypeStruct((S, D), A_x.dtype),
        in_specs=[pl.BlockSpec(memory_space=pl.ANY)] * 6,
        out_specs=pl.BlockSpec(memory_space=pl.ANY),
        scratch_shapes=[
            pltpu.VMEM((S, D), BF16),
            pltpu.VMEM((D, D), BF16),
            pltpu.VMEM((NG + len(CROSS), S // 2, LANE), I32),
            pltpu.VMEM((H, LANE // 2, S), I32),
            pltpu.VMEM((NT, H * QR, LANE), F32),
            pltpu.VMEM((D, LANE, LANE), F32),
            pltpu.VMEM((H, VR, S), F32),
            pltpu.VMEM((H, N_EARLY, S), F32),
            pltpu.VMEM((H, 1, S), F32),
            pltpu.VMEM((3, D, D), BF16),
            pltpu.VMEM((D, F), BF16),
            pltpu.VMEM((D, F), BF16),
            pltpu.VMEM((F, D), BF16),
            pltpu.VMEM((S // 2, D), I32),
            pltpu.VMEM((2, LANE, D), F32),
            pltpu.VMEM((2, H, VR, LANE), F32),
            pltpu.VMEM((QT, S, LANE), F32),
            pltpu.VMEM((QT, S, LANE), F32),
            pltpu.VMEM((2, 8, BQ), F32),
            pltpu.VMEM((VR, BQ), F32),
            pltpu.SemaphoreType.DMA((S // XB,)),
            pltpu.SemaphoreType.DMA((7,)),
            pltpu.SemaphoreType.DMA((len(OB),)),
        ],
        compiler_params=pltpu.CompilerParams(vmem_limit_bytes=127 * 2**20),
    )(A_x.reshape(S, D), A_wqkv, A_wo, B_w_gate, B_w_up, B_w_down)
    return out.reshape(A_x.shape)
```

```python
import math

import jax
import jax.numpy as jnp
import numpy as np
from jax import lax
import jax.experimental.pallas as pl
import jax.experimental.pallas.tpu as pltpu

S, D, H, F = 2048, 640, 32, 1536
DH = D // H
LANE = 128
BQ = 512
KC = 128
NQ, NC, QT, NT, NG = S // BQ, S // KC, BQ // LANE, S // LANE, D // LANE
CROSS = [h for h in range(H) if DH * h // LANE != (DH * h + DH - 1) // LANE]
VR = 24
QR = 32
XB = 512
FB = 256
HB = H * FB // S
UH = 3
OB = (128, 128, 256, 256, 256, 256, 256, 256, 128, 128)

KV = 16
KM = KC - KV
EARLY = [c for c in range(NC) if c % 8 in (1, 3, 5)]
LIVE = [c for c in range(NC) if c not in EARLY]
N_EARLY, N_LIVE = KV * len(EARLY), KV * len(LIVE)
PACE = (1, 1, 1, 2, 3, 6, 2)

QSCALE = float(DH ** -0.5 * math.log2(math.e))
F32, BF16, I32 = jnp.float32, jnp.bfloat16, jnp.int32


def _dot(a, b):
    return lax.dot_general(a, b, (((1,), (0,)), ((), ())), preferred_element_type=F32)


def _after(value, other, true):
    if other.dtype != value.dtype:
        other = pltpu.bitcast(other, value.dtype)
    reps = (value.shape[0] // 8, value.shape[1] // LANE)
    if reps != (1, 1):
        true, other = jnp.tile(true, reps), jnp.tile(other, reps)
    return jnp.where(true, value, other)


def _outer(k, q):
    return k.reshape(1, k.shape[0] // 8, 8, LANE) * q[:, None]


def _lanes(t):
    return slice(t * LANE, (t + 1) * LANE)


def _cyclic(t, h):
    return jnp.concatenate([t[DH * h:DH * (h + 1)], t[DH * h:DH * h + QR - DH]], axis=0)


def _kernel(x_hbm, wqkv_hbm, wo_hbm, wg_hbm, wu_hbm, wd_hbm, out_hbm,
            x_v, wo_v, k_v, q_v, qf_v, kb_v, vt_v, es_v, em_v, wqkv_v, wg_v, wu_v, wd_v,
            xn_v, kf_v, kt_v, s0_v, s1_v, m_v, top_v, ot_v, xsems, wsems, osems):
    x_cp = [pltpu.make_async_copy(x_hbm.at[pl.ds(i * XB, XB)], x_v.at[pl.ds(i * XB, XB)], xsems.at[i])
            for i in range(S // XB)]
    wq_cp, wk_cp, wv_cp = [
        pltpu.make_async_copy(wqkv_hbm.at[:, pl.ds(i * D, D)], wqkv_v.at[i], wsems.at[i]) for i in range(3)]
    w_cp = [pltpu.make_async_copy(src, dst, wsems.at[3 + i]) for i, (src, dst) in enumerate(
        [(wg_hbm, wg_v), (wu_hbm, wu_v), (wd_hbm, wd_v), (wo_hbm, wo_v)])]

    def layernorm(lo, marks=(), true=None):
        n = 16 if marks else XB
        for j in range(XB // n):
            r = lo + n * j
            x = x_v[pl.ds(r, n), :]
            if marks:
                mark = marks[j * len(marks) // (XB // n)]
                x = pltpu.bitcast(_after(pltpu.bitcast(x, I32), mark, true), BF16)
            x = x.astype(F32)
            xc = x - jnp.mean(x, axis=-1, keepdims=True)
            var = jnp.mean(xc * xc, axis=-1, keepdims=True)
            xn_v[pl.ds(r // 2, n // 2), :] = pltpu.bitcast((xc * lax.rsqrt(var + 1e-5)).astype(BF16), I32)

    def project(which, lo, n, quartered):
        xn = pltpu.bitcast(xn_v[pl.ds(lo // 2, n // 2), :], BF16)
        if quartered:
            val = jnp.concatenate([
                _dot(xn, wqkv_v[which, :, 0:4 * LANE]),
                jnp.concatenate([_dot(xn[j * n // 4:(j + 1) * n // 4], wqkv_v[which, :, 4 * LANE:D])
                                 for j in range(4)], axis=0)], axis=1)
        else:
            val = _dot(xn, wqkv_v[which])
        return val, [val[r:r + 8, _lanes(g)] for g in range(NG) for r in range(0, n, 128)]

    def project_q(lo):
        val, marks = project(0, lo, XB, False)
        qt = (val * QSCALE).T
        row = lax.broadcasted_iota(I32, (LANE, XB), 0)
        groups = [qt[_lanes(g)] for g in range(NG)]
        groups += [jnp.where(row >= DH * h % LANE, groups[g], groups[g + 1]) for g, h in enumerate(CROSS)]
        for g, q in enumerate(groups):
            q_v[g, :, pl.ds(lo, XB)] = pltpu.bitcast(q.astype(BF16), I32)
        for h in range(H):
            ext = _cyclic(qt, h)
            for t in range(XB // LANE):
                qf_v[lo // LANE + t, QR * h:QR * (h + 1), :] = ext[:, _lanes(t)]
        return marks

    def project_k(lo, quartered=False):
        val, marks = project(1, lo, XB, quartered)
        lane = lax.broadcasted_iota(I32, (XB, LANE), 1)
        groups = [val[:, _lanes(g)] for g in range(NG)]
        groups += [jnp.where(lane >= DH * h % LANE, groups[g], groups[g + 1]) for g, h in enumerate(CROSS)]
        for g, k in enumerate(groups):
            k_v[g, pl.ds(lo // 2, XB // 2), :] = pltpu.bitcast(k.astype(BF16), I32)
        for c in range(lo // KC, (lo + XB) // KC):
            kf_v[pl.ds((EARLY + LIVE).index(c) * KV, KV), :] = val[c * KC - lo + KM:(c + 1) * KC - lo, :]
        return marks

    def project_v(lo, n=XB, quartered=False):
        val, marks = project(2, lo, n, quartered)
        vt = val.T
        row = lax.broadcasted_iota(I32, (VR, n), 0)
        for h in range(H):
            a = DH * h // 8 * 8
            r = DH * h - a
            vt_v[h, :, pl.ds(lo, n)] = jnp.where((row >= r) & (row < r + DH), vt[a:a + VR], 1.0)
        return marks

    def skew_keys(marks, true):
        sub = lax.broadcasted_iota(I32, (VR, LANE), 1) & 7
        for j in range(2):
            kt = kf_v[_lanes(j), :].T
            for h in range(H):
                ext = _after(_cyclic(kt, h), marks[(j * H + h) * len(marks) // (2 * H)], true)
                sk = ext[0:VR]
                for s in range(1, 8):
                    sk = jnp.where(sub == s, ext[s:s + VR], sk)
                kt_v[j, h] = sk

    def splat_keys(j, h, i):
        return jnp.broadcast_to(kt_v[j, h, i:i + 1, :], (LANE, LANE)).T

    def staged(j, i, first, n, zero=0):
        row = (i * N_EARLY + first) + zero * 8
        return j, pl.ds(row if isinstance(row, int) else pl.multiple_of(row, 8), n)

    def stage_keys(dst_v, j, h):
        for i in range(DH):
            kb = splat_keys(0, h, i)
            dst_v[staged(j, i, 0, N_EARLY)] = kb[:N_EARLY]
            kb_v[h * DH + i, 0:LANE - N_EARLY, :] = kb[N_EARLY:]

    def all_true():
        return (pltpu.bitcast(x_v[0:16, 0:LANE], I32) & 1) < 2

    x_cp[0].start()
    wk_cp.start()
    x_cp[0].wait()
    wv_cp.start()
    layernorm(0)
    wk_cp.wait()
    x_cp[1].start()
    project_k(0, quartered=True)
    wv_cp.wait()
    x_cp[1].wait()
    wq_cp.start()
    for cp in x_cp[2:]:
        cp.start()
    true = all_true()
    layernorm(XB, project_v(0)[:14], true)
    project_k(XB)
    project_v(XB, quartered=True)
    wq_cp.wait()
    for cp in x_cp[2:]:
        cp.wait()
    for cp in w_cp:
        cp.start()
    layernorm(2 * XB, (project_q(0) + project_q(XB))[:32], true)
    layernorm(3 * XB, (project_k(2 * XB) + project_v(2 * XB))[:32], true)
    project_k(3 * XB)
    skew_keys(project_q(2 * XB) + project_q(3 * XB), true)
    for j in range(HB):
        stage_keys(s0_v, j, j)
    project_v(3 * XB, XB - LANE)
    project_v(S - LANE, LANE)
    for cp in w_cp:
        cp.wait()

    def swiglu(blk, cur_v, nxt_v, zero):
        true = lax.broadcasted_iota(I32, (8, LANE), 0) >= -blk
        rows = pl.ds(pl.multiple_of(blk * FB, FB), FB)
        for j in range(HB):
            stage_keys(nxt_v, j, jnp.minimum(blk * HB + j + HB, H - 1))
        for j in range(HB):
            h = blk * HB + j
            for i in range(DH):
                kb_v[h * DH + i, LANE - N_EARLY:, :] = splat_keys(1, h, i)

        def early_scores():
            for j in range(HB):
                h = blk * HB + j
                for t in range(0, NT, 2):
                    top = None
                    for e in range(0, N_EARLY, 24):
                        for i in range(DH):
                            k = cur_v[staged(j, i, e, 24, zero)]
                            term = _outer(k, qf_v[t:t + 2, pl.ds(h * QR + i, 8), :])
                            acc = term if i == 0 else acc + term
                            yield acc
                        for u in range(2):
                            es_v[h, e:e + 24, _lanes(t + u)] = acc[u].reshape(24, LANE)
                        best = jnp.max(acc, axis=1)
                        top = best if top is None else jnp.maximum(top, best)
                    for u in range(2):
                        em_v[h, :, _lanes(t + u)] = jnp.max(top[u], axis=0, keepdims=True)

        side = early_scores()
        n_side = HB * N_EARLY // 24 * NT // 2 * DH
        n_slots = 3 * D * F // (4 * LANE * LANE) * FB // 16
        seen = dict(tile=0, slot=0, side=0)

        def paced_dot(a32, w):
            cols = []
            for g in range(a32.shape[1] // LANE):
                col = a32[:, _lanes(g)]
                if seen["tile"] % 4 == 0:
                    parts = []
                    for r in range(FB // 16):
                        seen["slot"] += 1
                        while seen["side"] < n_side * seen["slot"] // n_slots:
                            done = next(side)
                            seen["side"] += 1
                        parts.append(_after(col[r * 8:(r + 1) * 8], done[-1, -1], true))
                    col = jnp.concatenate(parts, axis=0)
                seen["tile"] += 1
                cols.append(col)
            return _dot(pltpu.bitcast(jnp.concatenate(cols, axis=1), BF16), w)

        xn = xn_v[pl.ds(pl.multiple_of(blk * (FB // 2), FB // 2), FB // 2), :]
        hidden = []
        for n in range(F // LANE):
            g = 0.5 * paced_dot(xn, wg_v[:, _lanes(n)])
            u = paced_dot(xn, wu_v[:, _lanes(n)])
            hidden.append(pltpu.bitcast(((g * jnp.tanh(g) + g) * u).astype(BF16), I32))
        hidden = jnp.concatenate(hidden, axis=1)
        x = x_v[rows, :]
        y = [(x[:, _lanes(n)].astype(F32) + paced_dot(hidden, wd_v[:, _lanes(n)])).astype(BF16)
             for n in range(NG)]
        for _ in side:
            pass
        x_v[rows, :] = jnp.concatenate(y, axis=1)

    def swiglu_pair(i, carry):
        swiglu(2 * i, s0_v, s1_v, 0)
        swiglu(2 * i + 1, s1_v, s0_v, i >> 16)
        return carry

    lax.fori_loop(0, S // FB // 2, swiglu_pair, 0)

    s_v = (s0_v, s1_v)

    def key_group(h):
        g0, g1 = h * DH // LANE, (h * DH + DH - 1) // LANE
        if isinstance(h, int):
            return g0 if g0 == g1 else NG + g0
        return jnp.where(g0 != g1, NG + g0, g0)

    def weigh_values(h, qb, c):
        cols = pl.ds(qb * BQ, BQ)
        keys = pl.ds(c * KC, KM if c in EARLY else KC)
        s = jnp.concatenate([s_v[qb % 2][t, keys, :] for t in range(QT)], axis=1)
        if c in EARLY:
            s = jnp.concatenate([s, es_v[h, pl.ds(EARLY.index(c) * KV, KV), cols]], axis=0)
        p = jnp.exp2(s.reshape(KC // 8, 8, BQ) - m_v[qb % 2][None]).reshape(KC, BQ).astype(BF16)
        ot = _dot(vt_v[h, :, pl.ds(c * KC, KC)], p)
        if c > 0:
            ot = ot_v[...] + ot
        if c < NC - 1:
            ot_v[...] = ot
        else:
            es_v[h, 0:VR, cols] = ot

    def step(h, qb, true, marks):
        cols = pl.ds(qb * BQ, BQ)
        g = key_group(h)
        top_live = {}

        def live_scores():
            for t in range(QT):
                for e in range(0, N_LIVE, 40):
                    for i in range(DH):
                        q = qf_v[qb * QT + t, pl.ds(h * QR + i, 8), :]
                        if i == 0 and len(marks) >= 5:
                            q = _after(q, marks[-5], true)
                        term = _outer(kb_v[h * DH + i, e:e + 40, :], q[None])[0]
                        acc = term if i == 0 else acc + term
                        for u in range(5):
                            yield acc, u
                    for u in range(5):
                        c, r = divmod(e + 8 * u, KV)
                        s_v[qb % 2][t, pl.ds(LIVE[c] * KC + KM + r, 8), :] = acc[u]
                        top_live[t] = jnp.maximum(top_live[t], acc[u]) if t in top_live else acc[u]

        side = live_scores()
        n_side = N_LIVE // 8 * QT * DH
        issued = slot = 0
        for c in range(NC):
            k32 = k_v[g, pl.ds(c * KC // 2, KM // 2), :]
            parts = []
            for r, share in enumerate(PACE):
                slot += share
                while issued < n_side * slot // (NC * sum(PACE)):
                    acc, u = next(side)
                    issued += 1
                parts.append(_after(k32[r * 8:(r + 1) * 8], acc[u], true))
            row = lax.broadcasted_iota(I32, (LANE, BQ), 0)
            qt = pltpu.bitcast(q_v[g, :, cols], BF16).astype(F32)
            qt = jnp.where(((row - h * DH) & (LANE - 1)) < DH, qt, 0.0).astype(BF16)
            st = _dot(pltpu.bitcast(jnp.concatenate(parts, axis=0), BF16), qt)
            for t in range(QT):
                s_v[qb % 2][t, pl.ds(c * KC, KM), :] = st[:, _lanes(t)]
            marks += [st[0:8, 0:LANE], st[64:72, 0:LANE]]
            top = jnp.max(st.reshape(KM // 8, 8, BQ), axis=0)
            if c > 0:
                top = jnp.maximum(top, top_v[...])
            if c < NC - 1:
                top_v[...] = top
            back = 1 if c > 0 else 2
            if qb >= back:
                weigh_values(h, qb - back, (c - 1) % NC)
            elif not (isinstance(h, int) and h == 0):
                weigh_values(h - 1, qb - back + NQ, (c - 1) % NC)
        for _ in side:
            pass
        top = jnp.maximum(top, jnp.concatenate([top_live[t] for t in range(QT)], axis=1))
        m = jnp.max(top, axis=0, keepdims=True)
        m_v[qb % 2] = jnp.broadcast_to(jnp.maximum(m, em_v[h, :, cols]), (8, BQ))

    def heads(h0, count, true):
        marks = []
        for u in range(count):
            for qb in range(NQ):
                step(h0 + u, qb, true, marks)

    def heads_body(i, carry):
        heads(1 + i * UH, UH, lax.broadcasted_iota(I32, (8, LANE), 0) >= -i)
        return carry

    heads(0, 1, all_true())
    lax.fori_loop(0, (H - 2) // UH, heads_body, 0)
    true = all_true()
    heads(H - 1, 1, true)

    start = np.concatenate([[0], np.cumsum(OB)]).tolist()
    o_cp = [pltpu.make_async_copy(x_v.at[pl.ds(start[i], n)], out_hbm.at[pl.ds(start[i], n)], osems.at[i])
            for i, n in enumerate(OB)]
    tail = [(NQ - 2, NC - 1)] + [(NQ - 1, c) for c in range(NC)]
    n_ready = len([end for end in start[1:] if end <= (NQ - 2) * BQ])
    mark = None
    for i, n in enumerate(OB):
        rows = pl.ds(start[i], n)
        low = lax.broadcasted_iota(I32, (8, n), 0) < 4
        parts = []
        for h in range(0, H, 2):
            a, b = es_v[h, 0:VR, rows], es_v[h + 1, 0:VR, rows]
            den = jnp.where(low, b[0:8], a[16:24])
            if mark is not None:
                den = _after(den, mark, true)
            inv = 1.0 / den
            ia, ib = jnp.broadcast_to(inv[7:8], (8, n)), jnp.broadcast_to(inv[0:1], (8, n))
            parts += [a[0:8] * ia, a[8:16] * ia, jnp.where(low, a[16:24] * ia, b[0:8] * ib),
                      b[8:16] * ib, b[16:24] * ib]
        res = _dot(jnp.concatenate(parts, axis=0).T.astype(BF16), wo_v[...])
        mark = res[0:8, 0:LANE]
        x_v[rows, :] = (x_v[rows, :].astype(F32) + res).astype(BF16)
        o_cp[i].start()
        if i < n_ready:
            for qb, c in tail[i * len(tail) // n_ready:(i + 1) * len(tail) // n_ready]:
                weigh_values(H - 1, qb, c)
    for cp in o_cp:
        cp.wait()


@jax.jit
def pallas_parallel_sum__mha_block__swiglu_ffn__prompt_kernel(
    A_x: jax.Array,
    A_wqkv: jax.Array,
    A_wo: jax.Array,
    B_x: jax.Array,
    B_w_gate: jax.Array,
    B_w_up: jax.Array,
    B_w_down: jax.Array,
):
    del B_x
    out = pl.pallas_call(
        _kernel,
        out_shape=jax.ShapeDtypeStruct((S, D), A_x.dtype),
        in_specs=[pl.BlockSpec(memory_space=pl.ANY)] * 6,
        out_specs=pl.BlockSpec(memory_space=pl.ANY),
        scratch_shapes=[
            pltpu.VMEM((S, D), BF16),
            pltpu.VMEM((D, D), BF16),
            pltpu.VMEM((NG + len(CROSS), S // 2, LANE), I32),
            pltpu.VMEM((NG + len(CROSS), LANE // 2, S), I32),
            pltpu.VMEM((NT, H * QR, LANE), F32),
            pltpu.VMEM((D, N_LIVE, LANE), F32),
            pltpu.VMEM((H, VR, S), F32),
            pltpu.VMEM((H, N_EARLY, S), F32),
            pltpu.VMEM((H, 1, S), F32),
            pltpu.VMEM((3, D, D), BF16),
            pltpu.VMEM((D, F), BF16),
            pltpu.VMEM((D, F), BF16),
            pltpu.VMEM((F, D), BF16),
            pltpu.VMEM((S // 2, D), I32),
            pltpu.VMEM((2 * LANE, D), F32),
            pltpu.VMEM((2, H, VR, LANE), F32),
            pltpu.VMEM((QT, S, LANE), F32),
            pltpu.VMEM((QT, S, LANE), F32),
            pltpu.VMEM((2, 8, BQ), F32),
            pltpu.VMEM((8, BQ), F32),
            pltpu.VMEM((VR, BQ), F32),
            pltpu.SemaphoreType.DMA((S // XB,)),
            pltpu.SemaphoreType.DMA((7,)),
            pltpu.SemaphoreType.DMA((len(OB),)),
        ],
        compiler_params=pltpu.CompilerParams(vmem_limit_bytes=127 * 2**20),
    )(A_x.reshape(S, D), A_wqkv, A_wo, B_w_gate, B_w_up, B_w_down)
    return out.reshape(A_x.shape)
```

```python
import math

import jax
import jax.numpy as jnp
import numpy as np
from jax import lax
import jax.experimental.pallas as pl
import jax.experimental.pallas.tpu as pltpu

S, D, H, F = 2048, 640, 32, 1536
DH = D // H
LANE = 128
BQ = 512
KC = 128
NQ, NC, QT, NT, NG = S // BQ, S // KC, BQ // LANE, S // LANE, D // LANE
CROSS = [h for h in range(H) if DH * h // LANE != (DH * h + DH - 1) // LANE]
VR = 24
QR = 32
XB = 512
FB = 256
HB = H * FB // S
UH = 2
OB = (128, 128, 256, 256, 256, 256, 256, 256, 128, 128)

KV = 16
KM = KC - KV
EARLY = [c for c in range(NC) if c % 8 in (1, 3, 5)]
LIVE = [c for c in range(NC) if c not in EARLY]
N_EARLY, N_LIVE = KV * len(EARLY), KV * len(LIVE)
PACE = (1, 1, 2, 2, 3, 6, 2)

QSCALE = float(DH ** -0.5 * math.log2(math.e))
F32, BF16, I32 = jnp.float32, jnp.bfloat16, jnp.int32


def _dot(a, b):
    return lax.dot_general(a, b, (((1,), (0,)), ((), ())), preferred_element_type=F32)


def _after(value, other, true):
    if other.dtype != value.dtype:
        other = pltpu.bitcast(other, value.dtype)
    reps = (value.shape[0] // 8, value.shape[1] // LANE)
    if reps != (1, 1):
        true, other = jnp.tile(true, reps), jnp.tile(other, reps)
    return jnp.where(true, value, other)


def _lanes(t):
    return slice(t * LANE, (t + 1) * LANE)


def _cyclic(t, h):
    return jnp.concatenate([t[DH * h:DH * (h + 1)], t[DH * h:DH * h + QR - DH]], axis=0)


def _kernel(x_hbm, wqkv_hbm, wo_hbm, wg_hbm, wu_hbm, wd_hbm, out_hbm,
            x_v, wo_v, k_v, q_v, qf_v, kb_v, vt_v, es_v, em_v, wqkv_v, wg_v, wu_v, wd_v,
            xn_v, kf_v, kt_v, s0_v, s1_v, m_v, top_v, ot_v, xsems, wsems, osems):
    x_cp = [pltpu.make_async_copy(x_hbm.at[pl.ds(i * XB, XB)], x_v.at[pl.ds(i * XB, XB)], xsems.at[i])
            for i in range(S // XB)]
    wq_cp, wk_cp, wv_cp = [
        pltpu.make_async_copy(wqkv_hbm.at[:, pl.ds(i * D, D)], wqkv_v.at[i], wsems.at[i]) for i in range(3)]
    *w_cp, wo_cp = [pltpu.make_async_copy(src, dst, wsems.at[3 + i]) for i, (src, dst) in enumerate(
        [(wg_hbm, wg_v), (wu_hbm, wu_v), (wd_hbm, wd_v), (wo_hbm, wo_v)])]

    def layernorm(lo, marks=(), true=None):
        n = 16 if marks else XB
        for j in range(XB // n):
            r = lo + n * j
            x = x_v[pl.ds(r, n), :]
            if marks:
                mark = marks[j * len(marks) // (XB // n)]
                x = pltpu.bitcast(_after(pltpu.bitcast(x, I32), mark, true), BF16)
            x = x.astype(F32)
            xc = x - jnp.mean(x, axis=-1, keepdims=True)
            var = jnp.mean(xc * xc, axis=-1, keepdims=True)
            xn_v[pl.ds(r // 2, n // 2), :] = pltpu.bitcast((xc * lax.rsqrt(var + 1e-5)).astype(BF16), I32)

    def project(which, lo, n, quartered):
        xn = pltpu.bitcast(xn_v[pl.ds(lo // 2, n // 2), :], BF16)
        if quartered:
            val = jnp.concatenate([
                _dot(xn, wqkv_v[which, :, 0:4 * LANE]),
                jnp.concatenate([_dot(xn[j * n // 4:(j + 1) * n // 4], wqkv_v[which, :, 4 * LANE:D])
                                 for j in range(4)], axis=0)], axis=1)
        else:
            val = _dot(xn, wqkv_v[which])
        return val, [val[r:r + 8, _lanes(g)] for g in range(NG) for r in range(0, n, 128)]

    def project_q(lo):
        val, marks = project(0, lo, XB, False)
        qt = (val * QSCALE).T
        row = lax.broadcasted_iota(I32, (LANE, XB), 0)
        groups = [qt[_lanes(g)] for g in range(NG)]
        groups += [jnp.where(row >= DH * h % LANE, groups[g], groups[g + 1]) for g, h in enumerate(CROSS)]
        for g, q in enumerate(groups):
            q_v[g, :, pl.ds(lo, XB)] = pltpu.bitcast(q.astype(BF16), I32)
        for h in range(H):
            ext = _cyclic(qt, h)
            for t in range(XB // LANE):
                qf_v[lo // LANE + t, QR * h:QR * (h + 1), :] = ext[:, _lanes(t)]
        return marks

    def project_k(lo, quartered=False):
        val, marks = project(1, lo, XB, quartered)
        lane = lax.broadcasted_iota(I32, (XB, LANE), 1)
        groups = [val[:, _lanes(g)] for g in range(NG)]
        groups += [jnp.where(lane >= DH * h % LANE, groups[g], groups[g + 1]) for g, h in enumerate(CROSS)]
        for g, k in enumerate(groups):
            k_v[g, pl.ds(lo // 2, XB // 2), :] = pltpu.bitcast(k.astype(BF16), I32)
        for c in range(lo // KC, (lo + XB) // KC):
            kf_v[pl.ds((EARLY + LIVE).index(c) * KV, KV), :] = val[c * KC - lo + KM:(c + 1) * KC - lo, :]
        return marks

    def project_v(lo, n=XB, quartered=False):
        val, marks = project(2, lo, n, quartered)
        vt = val.T
        row = lax.broadcasted_iota(I32, (VR, n), 0)
        for h in range(H):
            a = DH * h // 8 * 8
            r = DH * h - a
            vt_v[h, :, pl.ds(lo, n)] = jnp.where((row >= r) & (row < r + DH), vt[a:a + VR], 1.0)
        return marks

    def skew_keys(marks, true):
        sub = lax.broadcasted_iota(I32, (VR, LANE), 1) & 7
        for j in range(2):
            kt = kf_v[_lanes(j), :].T
            for h in range(H):
                ext = _after(_cyclic(kt, h), marks[(j * H + h) * len(marks) // (2 * H)], true)
                sk = ext[0:VR]
                for s in range(1, 8):
                    sk = jnp.where(sub == s, ext[s:s + VR], sk)
                kt_v[j, h] = sk

    def splat_keys(j, h, i):
        return jnp.broadcast_to(kt_v[j, h, i:i + 1, :], (LANE, LANE)).T

    def stage_keys(dst_v, j, h):
        for i in range(DH):
            kb = splat_keys(0, h, i)
            dst_v[j, pl.ds(i * N_EARLY, N_EARLY), :] = kb[:N_EARLY]
            kb_v[h * DH + i, 0:LANE - N_EARLY, :] = kb[N_EARLY:]

    def all_true():
        return (pltpu.bitcast(x_v[0:16, 0:LANE], I32) & 1) < 2

    x_cp[0].start()
    wk_cp.start()
    x_cp[0].wait()
    wv_cp.start()
    layernorm(0)
    wk_cp.wait()
    x_cp[1].start()
    project_k(0, quartered=True)
    wv_cp.wait()
    x_cp[1].wait()
    wq_cp.start()
    for cp in x_cp[2:]:
        cp.start()
    true = all_true()
    layernorm(XB, project_v(0)[:14], true)
    project_k(XB)
    project_v(XB, quartered=True)
    wq_cp.wait()
    for cp in x_cp[2:]:
        cp.wait()
    for cp in w_cp:
        cp.start()
    layernorm(2 * XB, (project_q(0) + project_q(XB))[:32], true)
    layernorm(3 * XB, (project_k(2 * XB) + project_v(2 * XB))[:32], true)
    project_k(3 * XB)
    skew_keys(project_q(2 * XB) + project_q(3 * XB), true)
    for j in range(HB):
        stage_keys(s0_v, j, j)
    project_v(3 * XB, XB - LANE)
    project_v(S - LANE, LANE)
    for cp in w_cp:
        cp.wait()

    def swiglu(blk, cur_v, nxt_v, zero):
        true = lax.broadcasted_iota(I32, (8, LANE), 0) >= -blk
        rows = pl.ds(pl.multiple_of(blk * FB, FB), FB)
        for j in range(HB):
            stage_keys(nxt_v, j, jnp.minimum(blk * HB + j + HB, H - 1))
        for j in range(HB):
            h = blk * HB + j
            for i in range(DH):
                kb_v[h * DH + i, LANE - N_EARLY:, :] = splat_keys(1, h, i)

        def early_scores():
            k_rows = {(i, e): pl.ds(pl.multiple_of(i * N_EARLY + e + zero * 8, 8), 24)
                      for i in range(DH) for e in range(0, N_EARLY, 24)}
            for j in range(HB):
                h = blk * HB + j
                q_rows = [pl.ds(h * QR + i, 8) for i in range(DH)]
                for t in range(0, NT, 2):
                    top = None
                    for e in range(0, N_EARLY, 24):
                        for i in range(DH):
                            k = cur_v[j, k_rows[i, e], :].reshape(1, 3, 8, LANE)
                            term = k * qf_v[t:t + 2, q_rows[i], :][:, None]
                            acc = term if i == 0 else acc + term
                            yield acc
                        for u in range(2):
                            es_v[h, e:e + 24, _lanes(t + u)] = acc[u].reshape(24, LANE)
                        best = jnp.max(acc, axis=1)
                        top = best if top is None else jnp.maximum(top, best)
                    for u in range(2):
                        em_v[h, :, _lanes(t + u)] = jnp.max(top[u], axis=0, keepdims=True)

        side = early_scores()
        n_side = HB * N_EARLY // 24 * NT // 2 * DH
        n_slots = 3 * D * F // (4 * LANE * LANE) * FB // 16
        seen = dict(tile=0, slot=0, side=0)

        def paced_dot(a32, w):
            cols = []
            for g in range(a32.shape[1] // LANE):
                col = a32[:, _lanes(g)]
                if seen["tile"] % 4 == 0:
                    parts = []
                    for r in range(FB // 16):
                        seen["slot"] += 1
                        while seen["side"] < n_side * seen["slot"] // n_slots:
                            done = next(side)
                            seen["side"] += 1
                        parts.append(_after(col[r * 8:(r + 1) * 8], done[-1, -1], true))
                    col = jnp.concatenate(parts, axis=0)
                seen["tile"] += 1
                cols.append(col)
            return _dot(pltpu.bitcast(jnp.concatenate(cols, axis=1), BF16), w)

        xn = xn_v[pl.ds(pl.multiple_of(blk * (FB // 2), FB // 2), FB // 2), :]
        hidden = []
        for n in range(F // LANE):
            g = 0.5 * paced_dot(xn, wg_v[:, _lanes(n)])
            u = paced_dot(xn, wu_v[:, _lanes(n)])
            hidden.append(pltpu.bitcast(((g * jnp.tanh(g) + g) * u).astype(BF16), I32))
        hidden = jnp.concatenate(hidden, axis=1)
        x = x_v[rows, :]
        y = [(x[:, _lanes(n)].astype(F32) + paced_dot(hidden, wd_v[:, _lanes(n)])).astype(BF16)
             for n in range(NG)]
        for _ in side:
            pass
        x_v[rows, :] = jnp.concatenate(y, axis=1)

    def swiglu_pair(i, carry):
        swiglu(2 * i, s0_v, s1_v, 0)
        swiglu(2 * i + 1, s1_v, s0_v, i >> 16)
        return carry

    lax.fori_loop(0, S // FB // 2, swiglu_pair, 0)

    s_v = (s0_v, s1_v)

    def key_group(h):
        g0, g1 = h * DH // LANE, (h * DH + DH - 1) // LANE
        if isinstance(h, int):
            return g0 if g0 == g1 else NG + g0
        return jnp.where(g0 != g1, NG + g0, g0)

    def weigh_values(h, qb, c):
        cols = pl.ds(qb * BQ, BQ)
        keys = pl.ds(c * KC, KM if c in EARLY else KC)
        s = jnp.concatenate([s_v[qb % 2][t, keys, :] for t in range(QT)], axis=1)
        if c in EARLY:
            s = jnp.concatenate([s, es_v[h, pl.ds(EARLY.index(c) * KV, KV), cols]], axis=0)
        p = jnp.exp2(s.reshape(KC // 8, 8, BQ) - m_v[qb % 2][None]).reshape(KC, BQ).astype(BF16)
        ot = _dot(vt_v[h, :, pl.ds(c * KC, KC)], p)
        if c > 0:
            ot = ot_v[...] + ot
        if c < NC - 1:
            ot_v[...] = ot
        else:
            es_v[h, 0:VR, cols] = ot

    def step(h, qb, true, marks):
        cols = pl.ds(qb * BQ, BQ)
        g = key_group(h)
        q_rows = [pl.ds(h * QR + i, 8) for i in range(DH)]
        k_rows = [h * DH + i for i in range(DH)]
        top_live = {}

        def live_scores():
            for t in range(QT):
                for e in range(0, N_LIVE, 40):
                    for i in range(DH):
                        q = qf_v[qb * QT + t, q_rows[i], :]
                        if i == 0 and len(marks) >= 5:
                            q = _after(q, marks[-5], true)
                        term = kb_v[k_rows[i], e:e + 40, :].reshape(5, 8, LANE) * q[None]
                        acc = term if i == 0 else acc + term
                        for u in range(5):
                            yield acc, u
                    for u in range(5):
                        c, r = divmod(e + 8 * u, KV)
                        s_v[qb % 2][t, pl.ds(LIVE[c] * KC + KM + r, 8), :] = acc[u]
                        top_live[t] = jnp.maximum(top_live[t], acc[u]) if t in top_live else acc[u]

        side = live_scores()
        n_side = N_LIVE // 8 * QT * DH
        issued = slot = 0
        for c in range(NC):
            k32 = k_v[g, pl.ds(c * KC // 2, KM // 2), :]
            parts = []
            for r, share in enumerate(PACE):
                slot += share
                while issued < n_side * slot // (NC * sum(PACE)):
                    acc, u = next(side)
                    issued += 1
                parts.append(_after(k32[r * 8:(r + 1) * 8], acc[u], true))
            row = lax.broadcasted_iota(I32, (LANE, BQ), 0)
            qt = pltpu.bitcast(q_v[g, :, cols], BF16).astype(F32)
            qt = jnp.where(((row - h * DH) & (LANE - 1)) < DH, qt, 0.0).astype(BF16)
            st = _dot(pltpu.bitcast(jnp.concatenate(parts, axis=0), BF16), qt)
            for t in range(QT):
                s_v[qb % 2][t, pl.ds(c * KC, KM), :] = st[:, _lanes(t)]
            marks += [st[0:8, 0:LANE], st[64:72, 0:LANE]]
            top = jnp.max(st.reshape(KM // 8, 8, BQ), axis=0)
            if c > 0:
                top = jnp.maximum(top, top_v[...])
            if c < NC - 1:
                top_v[...] = top
            back = 1 if c > 0 else 2
            if qb >= back:
                weigh_values(h, qb - back, (c - 1) % NC)
            elif not (isinstance(h, int) and h == 0):
                weigh_values(h - 1, qb - back + NQ, (c - 1) % NC)
        for _ in side:
            pass
        top = jnp.maximum(top, jnp.concatenate([top_live[t] for t in range(QT)], axis=1))
        m = jnp.max(top, axis=0, keepdims=True)
        m_v[qb % 2] = jnp.broadcast_to(jnp.maximum(m, em_v[h, :, cols]), (8, BQ))

    def heads(h0, count, true):
        marks = []
        for u in range(count):
            for qb in range(NQ):
                step(h0 + u, qb, true, marks)

    def heads_body(i, carry):
        heads(1 + i * UH, UH, lax.broadcasted_iota(I32, (8, LANE), 0) >= -i)
        return carry

    wo_cp.start()
    heads(0, 1, all_true())
    lax.fori_loop(0, (H - 2) // UH, heads_body, 0)
    wo_cp.wait()
    true = all_true()
    heads(H - 1, 1, true)

    start = np.concatenate([[0], np.cumsum(OB)]).tolist()
    o_cp = [pltpu.make_async_copy(x_v.at[pl.ds(start[i], n)], out_hbm.at[pl.ds(start[i], n)], osems.at[i])
            for i, n in enumerate(OB)]
    tail = [(NQ - 2, NC - 1)] + [(NQ - 1, c) for c in range(NC)]
    n_ready = len([end for end in start[1:] if end <= (NQ - 2) * BQ])
    mark = None
    for i, n in enumerate(OB):
        rows = pl.ds(start[i], n)
        low = lax.broadcasted_iota(I32, (8, n), 0) < 4
        parts = []
        for h in range(0, H, 2):
            a, b = es_v[h, 0:VR, rows], es_v[h + 1, 0:VR, rows]
            den = jnp.where(low, b[0:8], a[16:24])
            if mark is not None:
                den = _after(den, mark, true)
            inv = 1.0 / den
            ia, ib = jnp.broadcast_to(inv[7:8], (8, n)), jnp.broadcast_to(inv[0:1], (8, n))
            parts += [a[0:8] * ia, a[8:16] * ia, jnp.where(low, a[16:24] * ia, b[0:8] * ib),
                      b[8:16] * ib, b[16:24] * ib]
        res = _dot(jnp.concatenate(parts, axis=0).T.astype(BF16), wo_v[...])
        mark = res[0:8, 0:LANE]
        x_v[rows, :] = (x_v[rows, :].astype(F32) + res).astype(BF16)
        o_cp[i].start()
        if i < n_ready:
            for qb, c in tail[i * len(tail) // n_ready:(i + 1) * len(tail) // n_ready]:
                weigh_values(H - 1, qb, c)
    for cp in o_cp:
        cp.wait()


@jax.jit
def pallas_parallel_sum__mha_block__swiglu_ffn__prompt_kernel(
    A_x: jax.Array,
    A_wqkv: jax.Array,
    A_wo: jax.Array,
    B_x: jax.Array,
    B_w_gate: jax.Array,
    B_w_up: jax.Array,
    B_w_down: jax.Array,
):
    del B_x
    out = pl.pallas_call(
        _kernel,
        out_shape=jax.ShapeDtypeStruct((S, D), A_x.dtype),
        in_specs=[pl.BlockSpec(memory_space=pl.ANY)] * 6,
        out_specs=pl.BlockSpec(memory_space=pl.ANY),
        scratch_shapes=[
            pltpu.VMEM((S, D), BF16),
            pltpu.VMEM((D, D), BF16),
            pltpu.VMEM((NG + len(CROSS), S // 2, LANE), I32),
            pltpu.VMEM((NG + len(CROSS), LANE // 2, S), I32),
            pltpu.VMEM((NT, H * QR, LANE), F32),
            pltpu.VMEM((D, N_LIVE, LANE), F32),
            pltpu.VMEM((H, VR, S), F32),
            pltpu.VMEM((H, N_EARLY, S), F32),
            pltpu.VMEM((H, 1, S), F32),
            pltpu.VMEM((3, D, D), BF16),
            pltpu.VMEM((D, F), BF16),
            pltpu.VMEM((D, F), BF16),
            pltpu.VMEM((F, D), BF16),
            pltpu.VMEM((S // 2, D), I32),
            pltpu.VMEM((2 * LANE, D), F32),
            pltpu.VMEM((2, H, VR, LANE), F32),
            pltpu.VMEM((QT, S, LANE), F32),
            pltpu.VMEM((QT, S, LANE), F32),
            pltpu.VMEM((2, 8, BQ), F32),
            pltpu.VMEM((8, BQ), F32),
            pltpu.VMEM((VR, BQ), F32),
            pltpu.SemaphoreType.DMA((S // XB,)),
            pltpu.SemaphoreType.DMA((7,)),
            pltpu.SemaphoreType.DMA((len(OB),)),
        ],
        compiler_params=pltpu.CompilerParams(vmem_limit_bytes=127 * 2**20),
    )(A_x.reshape(S, D), A_wqkv, A_wo, B_w_gate, B_w_up, B_w_down)
    return out.reshape(A_x.shape)
```
